```python
import os as _os
_os.environ.setdefault("JAX_PLATFORMS", "cpu")
import jax
import jax.numpy as jnp

def _softmax(x, axis=-1):
    return jax.nn.softmax(x, axis=axis)
def _gelu(x):
    return jax.nn.gelu(x, approximate=True)
def _silu(x):
    return jax.nn.silu(x)
def _sigmoid(x):
    return jax.nn.sigmoid(x)
def _layernorm(x, axis=-1, eps=1e-5):
    m = jnp.mean(x, axis=axis, keepdims=True)
    v = jnp.var(x, axis=axis, keepdims=True)
    return (x - m) / jnp.sqrt(v + eps)
def _scatter_add(tgt, idx, src, axis=0):
    return tgt.at[idx].add(src)
def _segment_sum(src, seg, n):
    return jax.ops.segment_sum(src, seg, n)
class _Rng:
    def __init__(self, key):
        self._k = key
    def _next(self):
        self._k, sub = jax.random.split(self._k)
        return sub
    def normal(self, shape):
        return jax.random.normal(self._next(), shape, dtype=jnp.bfloat16)
    def randint(self, lo, hi, shape):
        return jax.random.randint(self._next(), shape, lo, hi, dtype=jnp.int32)
    def uniform(self, shape, lo=0.0, hi=1.0):
        return jax.random.uniform(self._next(), shape, jnp.bfloat16, lo, hi)
    def permutation(self, n):
        return jax.random.permutation(self._next(), n)


kernel_name = 'concat_heads__mha_block_cached__gqa_block_cached__near_ridge'

def setup_inputs():
    _rng = _Rng(jax.random.key(int.from_bytes(__import__("os").urandom(4), "little")))
    _w = (lambda a: (lambda t: t.astype(jnp.bfloat16) if jnp.issubdtype(t.dtype, jnp.floating) else t)(jnp.asarray(a)))
    def _A_setup():
        B, Sq, D = 8, 128, 512
        H, Sk, Dh = 32, 1024, 128
        return {
            "x": _w((lambda *s: _rng.normal(s) * 0.8)(B, Sq, D)),
            "k_cache": _w((lambda *s: _rng.normal(s) * 0.8)(B, H, Sk, Dh)),
            "v_cache": _w((lambda *s: _rng.normal(s) * 0.05)(B, H, Sk, Dh)),
            "wq": _w((lambda *s: _rng.normal(s) * 0.8)(D, H * Dh) * (D ** -0.5)),
            "wo": _w((lambda *s: _rng.normal(s) * 0.05)(H * Dh, D) * ((H * Dh) ** -0.5)),
        }
    _A_in = _A_setup()

    def _B_setup():
        B, Sq, D = 8, 128, 512
        Hq, Hkv, Sk, Dh = 32, 32, 1024, 128
        assert Hq % Hkv == 0, (Hq, Hkv)
        return {
            "x": _w((lambda *s: _rng.normal(s) * 0.8)(B, Sq, D)),
            "k_cache": _w((lambda *s: _rng.normal(s) * 0.8)(B, Hkv, Sk, Dh)),
            "v_cache": _w((lambda *s: _rng.normal(s) * 0.05)(B, Hkv, Sk, Dh)),
            "wq": _w((lambda *s: _rng.normal(s) * 0.8)(D, Hq * Dh) * (D ** -0.5)),
            "wo": _w((lambda *s: _rng.normal(s) * 0.05)(Hq * Dh, D) * ((Hq * Dh) ** -0.5)),
        }
    _B_in = _B_setup()

    return {
        "A_x": _A_in["x"],
        "A_k_cache": _A_in["k_cache"],
        "A_v_cache": _A_in["v_cache"],
        "A_wq": _A_in["wq"],
        "A_wo": _A_in["wo"],
        "B_x": _B_in["x"],
        "B_k_cache": _B_in["k_cache"],
        "B_v_cache": _B_in["v_cache"],
        "B_wq": _B_in["wq"],
        "B_wo": _B_in["wo"],
    }

def reference(A_x, A_k_cache, A_v_cache, A_wq, A_wo, B_x, B_k_cache, B_v_cache, B_wq, B_wo):
    def _A_ref(x, k_cache, v_cache, wq, wo):
        B, Sq, D = x.shape
        H, Dh = 32, 128
        q = (lambda x, *d: x.transpose(*d))((x @ wq).reshape(B, Sq, H, Dh), 0, 2, 1, 3)
        scores = jnp.einsum("bhqd,bhkd->bhqk", q, k_cache) * (Dh ** -0.5)
        p = _softmax(scores, axis=-1)
        o = jnp.einsum("bhqk,bhkd->bhqd", p, v_cache)
        return (lambda x, *d: x.transpose(*d))(o, 0, 2, 1, 3).reshape(B, Sq, H * Dh) @ wo

    def _B_ref(x, k_cache, v_cache, wq, wo):
        B, Sq, D = x.shape
        Hq, Dh = 32, 128
        Hkv = k_cache.shape[1]
        rep = Hq // Hkv
        q = (lambda x, *d: x.transpose(*d))((x @ wq).reshape(B, Sq, Hq, Dh), 0, 2, 1, 3)
        k = jnp.repeat(k_cache, rep, axis=1)
        v = jnp.repeat(v_cache, rep, axis=1)
        scores = jnp.einsum("bhqd,bhkd->bhqk", q, k) * (Dh ** -0.5)
        p = _softmax(scores, axis=-1)
        o = jnp.einsum("bhqk,bhkd->bhqd", p, v)
        return (lambda x, *d: x.transpose(*d))(o, 0, 2, 1, 3).reshape(B, Sq, Hq * Dh) @ wo

    a = _A_ref(A_x, A_k_cache, A_v_cache, A_wq, A_wo)
    b = _B_ref(B_x, B_k_cache, B_v_cache, B_wq, B_wo)
    return jnp.concatenate([a, b], axis=-1)
```

```python
import math
import jax
import jax.numpy as jnp
from jax import lax
import jax.experimental.pallas as pl
import jax.experimental.pallas.tpu as pltpu

PD = 2
NS = PD + 1
FINE = 0
Dh = 128
H = 32
NB = 8
NT = NB * H
QSCALE = (Dh ** -0.5) * math.log2(math.e)


def kernel(ax, ak, av, awq, awo, bx, bk, bv, bwq, bwo, out_hbm,
           x_buf, wq_buf, wo_buf, k_buf, v_buf, s_buf, acc, o_stage,
           wsem, ksem, vsem, osem):
    xs, ks, vs, wqs, wos = (ax, bx), (ak, bk), (av, bv), (awq, bwq), (awo, bwo)

    def kcopy(br, t):
        return pltpu.make_async_copy(ks[br].at[t // H, t % H], k_buf.at[t % NS, br], ksem.at[t % NS, br])

    def vcopy(br, t):
        return pltpu.make_async_copy(vs[br].at[t // H, t % H], v_buf.at[t % NS, br], vsem.at[t % NS, br])

    def xcopy(br):
        return pltpu.make_async_copy(xs[br], x_buf.at[br], wsem.at[br])

    def wqcopy(br):
        return pltpu.make_async_copy(wqs[br], wq_buf.at[br], wsem.at[2 + br])

    def wocopy(br):
        return pltpu.make_async_copy(wos[br], wo_buf.at[br], wsem.at[4 + br])

    def ocopy(b):
        return pltpu.make_async_copy(o_stage.at[b % 2], out_hbm.at[b], osem.at[b % 2])

    def issue(t):
        kcopy(1, t).start()
        if isinstance(t, int):
            if t + 1 < NT:
                kcopy(0, t + 1).start()
        else:
            @pl.when(t + 1 < NT)
            def _():
                kcopy(0, t + 1).start()
        vcopy(0, t).start()
        vcopy(1, t).start()

    def qk(br, t):
        x = x_buf[br, t // H]
        wq = wq_buf[br, :, pl.ds(pl.multiple_of((t % H) * Dh, Dh), Dh)]
        q = jnp.dot(x, wq, preferred_element_type=jnp.float32)
        q = (q * QSCALE).astype(jnp.bfloat16)
        k = k_buf[t % NS, br]
        return lax.dot_general(q, k, (((1,), (1,)), ((), ())), preferred_element_type=jnp.float32)

    def soft(s):
        m = jnp.max(s, axis=-1, keepdims=True)
        p = jnp.exp2(s - m)
        l = jnp.sum(p, axis=-1, keepdims=True)
        return p.astype(jnp.bfloat16), l

    def pv(br, t, p, l):
        v = v_buf[t % NS, br]
        o = jnp.dot(p, v, preferred_element_type=jnp.float32)
        o = (o * (1.0 / l)).astype(jnp.bfloat16)
        wo = wo_buf[br, pl.ds(pl.multiple_of((t % H) * Dh, Dh), Dh), :]
        c = jnp.dot(o, wo, preferred_element_type=jnp.float32)
        acc[:, br * 512:(br + 1) * 512] += c

    xcopy(0).start(); wqcopy(0).start()
    kcopy(0, 0).start()
    xcopy(1).start(); wqcopy(1).start()
    wocopy(0).start(); wocopy(1).start()
    for t in range(PD):
        issue(t)
    acc[...] = jnp.zeros_like(acc)
    xcopy(0).wait(); wqcopy(0).wait()
    kcopy(0, 0).wait()
    s_buf[...] = qk(0, 0)
    xcopy(1).wait(); wqcopy(1).wait()
    wocopy(0).wait(); wocopy(1).wait()

    def finish_batch(b):
        if isinstance(b, int):
            if b >= 2:
                ocopy(b - 2).wait()
        else:
            @pl.when(b >= 2)
            def _():
                ocopy(b - 2).wait()
        o_stage[b % 2] = acc[...].astype(o_stage.dtype)
        ocopy(b).start()
        acc[...] = jnp.zeros_like(acc)

    def body(t, last):
        if not last:
            @pl.when(t + PD < NT)
            def _():
                issue(t + PD)
        if not FINE:
            kcopy(1, t).wait()
            if not last:
                kcopy(0, t + 1).wait()
            vcopy(0, t).wait()
            vcopy(1, t).wait()
            s_a = s_buf[...]
            s_b = qk(1, t)
            p, l = soft(s_a)
            pv(0, t, p, l)
            if not last:
                s_buf[...] = qk(0, t + 1)
            p, l = soft(s_b)
            pv(1, t, p, l)
        else:
            kcopy(1, t).wait()
            vcopy(0, t).wait()
            s_a = s_buf[...]
            s_b = qk(1, t)
            p, l = soft(s_a)
            pv(0, t, p, l)
            if not last:
                kcopy(0, t + 1).wait()
            vcopy(1, t).wait()
            if not last:
                s_buf[...] = qk(0, t + 1)
            p, l = soft(s_b)
            pv(1, t, p, l)
        if last:
            finish_batch(NB - 1)
        else:
            @pl.when(t % H == H - 1)
            def _():
                finish_batch(t // H)

    def loop_body(t, carry):
        body(t, False)
        return carry

    lax.fori_loop(0, NT - 1, loop_body, 0)
    body(NT - 1, True)
    ocopy(NB - 2).wait()
    ocopy(NB - 1).wait()


@jax.jit
def pallas_concat_heads__mha_block_cached__gqa_block_cached__near_ridge_kernel(
    A_x, A_k_cache, A_v_cache, A_wq, A_wo, B_x, B_k_cache, B_v_cache, B_wq, B_wo):
    B, Sq, D = A_x.shape
    _, Hh, Sk, _ = A_k_cache.shape
    bf = jnp.bfloat16
    return pl.pallas_call(
        kernel,
        in_specs=[pl.BlockSpec(memory_space=pl.ANY)] * 10,
        out_specs=pl.BlockSpec(memory_space=pl.ANY),
        out_shape=jax.ShapeDtypeStruct((B, Sq, 2 * D), bf),
        scratch_shapes=[
            pltpu.VMEM((2, B, Sq, D), bf),
            pltpu.VMEM((2, D, Hh * Dh), bf),
            pltpu.VMEM((2, Hh * Dh, D), bf),
            pltpu.VMEM((NS, 2, Sk, Dh), bf),
            pltpu.VMEM((NS, 2, Sk, Dh), bf),
            pltpu.VMEM((Sq, Sk), jnp.float32),
            pltpu.VMEM((Sq, 2 * D), jnp.float32),
            pltpu.VMEM((2, Sq, 2 * D), bf),
            pltpu.SemaphoreType.DMA((6,)),
            pltpu.SemaphoreType.DMA((NS, 2)),
            pltpu.SemaphoreType.DMA((NS, 2)),
            pltpu.SemaphoreType.DMA((2,)),
        ],
        compiler_params=pltpu.CompilerParams(vmem_limit_bytes=100 * 1024 * 1024),
    )(A_x, A_k_cache, A_v_cache, A_wq, A_wo, B_x, B_k_cache, B_v_cache, B_wq, B_wo)
```

```python
import functools
import math

import jax
import jax.numpy as jnp
from jax import lax
import jax.experimental.pallas as pl
import jax.experimental.pallas.tpu as pltpu

_DH = 128
_PD = 2
_NS = _PD + 1


def _kernel(ax, ak, av, awq, awo, bx, bk, bv, bwq, bwo, out_hbm,
            x_buf, wq_buf, wo_buf, k_buf, v_buf, s_buf, acc, o_early, o_last,
            wsem, ksem, vsem, osem, *, nb, nh, d_model, reps):
    xs, ks, vs, wqs, wos = (ax, bx), (ak, bk), (av, bv), (awq, bwq), (awo, bwo)
    nt = nb * nh
    qscale = (_DH ** -0.5) * math.log2(math.e)

    def kv_head(br, t):
        h = t % nh
        return h if reps[br] == 1 else h // reps[br]

    def kcopy(br, t):
        return pltpu.make_async_copy(
            ks[br].at[t // nh, kv_head(br, t)], k_buf.at[t % _NS, br], ksem.at[t % _NS, br])

    def vcopy(br, t):
        return pltpu.make_async_copy(
            vs[br].at[t // nh, kv_head(br, t)], v_buf.at[t % _NS, br], vsem.at[t % _NS, br])

    def xcopy(br):
        return pltpu.make_async_copy(xs[br], x_buf.at[br], wsem.at[br])

    def wqcopy(br):
        return pltpu.make_async_copy(wqs[br], wq_buf.at[br], wsem.at[2 + br])

    def wocopy(br):
        return pltpu.make_async_copy(wos[br], wo_buf.at[br], wsem.at[4 + br])

    def ocopy_early():
        return pltpu.make_async_copy(o_early, out_hbm.at[pl.ds(0, nb - 1)], osem.at[0])

    def ocopy_last():
        return pltpu.make_async_copy(o_last, out_hbm.at[nb - 1], osem.at[1])

    def issue(t):
        kcopy(1, t).start()
        if isinstance(t, int):
            if t + 1 < nt:
                kcopy(0, t + 1).start()
        else:
            @pl.when(t + 1 < nt)
            def _():
                kcopy(0, t + 1).start()
        vcopy(0, t).start()
        vcopy(1, t).start()

    def head_cols(t):
        return pl.ds(pl.multiple_of((t % nh) * _DH, _DH), _DH)

    def scores(br, t):
        x = x_buf[br, t // nh]
        wq = wq_buf[br, :, head_cols(t)]
        q = jnp.dot(x, wq, preferred_element_type=jnp.float32)
        q = (q * qscale).astype(jnp.bfloat16)
        k = k_buf[t % _NS, br]
        return lax.dot_general(q, k, (((1,), (1,)), ((), ())),
                               preferred_element_type=jnp.float32)

    def attend(br, t, s):
        m = jnp.max(s, axis=-1, keepdims=True)
        p = jnp.exp2(s - m)
        l = jnp.sum(p, axis=-1, keepdims=True)
        v = v_buf[t % _NS, br]
        o = jnp.dot(p.astype(jnp.bfloat16), v, preferred_element_type=jnp.float32)
        o = (o * (1.0 / l)).astype(jnp.bfloat16)
        wo = wo_buf[br, head_cols(t), :]
        acc[:, br * d_model:(br + 1) * d_model] += jnp.dot(
            o, wo, preferred_element_type=jnp.float32)

    xcopy(0).start()
    wqcopy(0).start()
    kcopy(0, 0).start()
    xcopy(1).start()
    wqcopy(1).start()
    wocopy(0).start()
    wocopy(1).start()
    for t0 in range(_PD):
        issue(t0)
    acc[...] = jnp.zeros_like(acc)
    xcopy(0).wait()
    wqcopy(0).wait()
    kcopy(0, 0).wait()
    s_buf[...] = scores(0, 0)
    xcopy(1).wait()
    wqcopy(1).wait()
    wocopy(0).wait()
    wocopy(1).wait()

    def body(t, last):
        if not last:
            @pl.when(t + _PD < nt)
            def _():
                issue(t + _PD)

            @pl.when(t == nt - 2)
            def _():
                ocopy_early().start()

        kcopy(1, t).wait()
        if not last:
            kcopy(0, t + 1).wait()
        vcopy(0, t).wait()
        vcopy(1, t).wait()

        s_a = s_buf[...]
        s_b = scores(1, t)
        attend(0, t, s_a)
        if not last:
            s_buf[...] = scores(0, t + 1)
        attend(1, t, s_b)

        if last:
            o_last[...] = acc[...].astype(o_last.dtype)
            ocopy_last().start()
        else:
            @pl.when(t % nh == nh - 1)
            def _():
                o_early[t // nh] = acc[...].astype(o_early.dtype)
                acc[...] = jnp.zeros_like(acc)

    def loop_body(t, carry):
        body(t, False)
        return carry

    lax.fori_loop(0, nt - 1, loop_body, 0)
    body(nt - 1, True)
    ocopy_early().wait()
    ocopy_last().wait()


@jax.jit
def pallas_concat_heads__mha_block_cached__gqa_block_cached__near_ridge_kernel(
    A_x: jax.Array,
    A_k_cache: jax.Array,
    A_v_cache: jax.Array,
    A_wq: jax.Array,
    A_wo: jax.Array,
    B_x: jax.Array,
    B_k_cache: jax.Array,
    B_v_cache: jax.Array,
    B_wq: jax.Array,
    B_wo: jax.Array,
):
    nb, sq, d_model = A_x.shape
    sk = A_k_cache.shape[2]
    nh = A_wq.shape[1] // _DH
    assert B_x.shape == A_x.shape and B_wq.shape == A_wq.shape and B_wo.shape == A_wo.shape
    assert A_k_cache.shape == (nb, nh, sk, _DH) and A_v_cache.shape == A_k_cache.shape
    assert B_k_cache.shape[2:] == (sk, _DH) and B_v_cache.shape == B_k_cache.shape
    assert nh % B_k_cache.shape[1] == 0 and nb >= 2 and nh >= 2
    reps = (1, nh // B_k_cache.shape[1])
    dt = A_x.dtype

    kernel = functools.partial(_kernel, nb=nb, nh=nh, d_model=d_model, reps=reps)
    return pl.pallas_call(
        kernel,
        in_specs=[pl.BlockSpec(memory_space=pl.ANY)] * 10,
        out_specs=pl.BlockSpec(memory_space=pl.ANY),
        out_shape=jax.ShapeDtypeStruct((nb, sq, 2 * d_model), dt),
        scratch_shapes=[
            pltpu.VMEM((2, nb, sq, d_model), dt),
            pltpu.VMEM((2, d_model, nh * _DH), dt),
            pltpu.VMEM((2, nh * _DH, d_model), dt),
            pltpu.VMEM((_NS, 2, sk, _DH), dt),
            pltpu.VMEM((_NS, 2, sk, _DH), dt),
            pltpu.VMEM((sq, sk), jnp.float32),
            pltpu.VMEM((sq, 2 * d_model), jnp.float32),
            pltpu.VMEM((nb - 1, sq, 2 * d_model), dt),
            pltpu.VMEM((sq, 2 * d_model), dt),
            pltpu.SemaphoreType.DMA((6,)),
            pltpu.SemaphoreType.DMA((_NS, 2)),
            pltpu.SemaphoreType.DMA((_NS, 2)),
            pltpu.SemaphoreType.DMA((2,)),
        ],
        compiler_params=pltpu.CompilerParams(vmem_limit_bytes=64 * 1024 * 1024),
    )(A_x, A_k_cache, A_v_cache, A_wq, A_wo, B_x, B_k_cache, B_v_cache, B_wq, B_wo)
```

```python
import functools
import math

import jax
import jax.numpy as jnp
from jax import lax
import jax.experimental.pallas as pl
import jax.experimental.pallas.tpu as pltpu

_DH = 128
_PD = 2
_NS = _PD + 1


def _pieces(rows, want, align):
    n = want
    while n > 1 and rows % (n * align):
        n //= 2
    return n


def _kernel(ax, ak, av, awq, awo, bx, bk, bv, bwq, bwo, out_hbm,
            x_buf, wq_buf, wo_buf, k_buf, v_buf, s_buf, acc, o_early, o_last,
            wsem, ksem, vsem, osem, *, nb, nh, d_model, reps):
    xs, ks, vs, wqs, wos = (ax, bx), (ak, bk), (av, bv), (awq, bwq), (awo, bwo)
    nt = nb * nh
    qscale = (_DH ** -0.5) * math.log2(math.e)

    def kv_head(br, t):
        h = t % nh
        return h if reps[br] == 1 else h // reps[br]

    def kcopy(br, t):
        return pltpu.make_async_copy(
            ks[br].at[t // nh, kv_head(br, t)], k_buf.at[t % _NS, br], ksem.at[t % _NS, br])

    def vcopy(br, t):
        return pltpu.make_async_copy(
            vs[br].at[t // nh, kv_head(br, t)], v_buf.at[t % _NS, br], vsem.at[t % _NS, br])

    resident = {}
    for br in range(2):
        resident["x", br] = (xs[br], x_buf.at[br], wsem.at[br], _pieces(nb, 4, 1))
        resident["wq", br] = (wqs[br], wq_buf.at[br], wsem.at[2 + br], _pieces(d_model, 16, 16))
        resident["wo", br] = (wos[br], wo_buf.at[br], wsem.at[4 + br], _pieces(nh * _DH, 16, 16))

    def fetch(*key):
        src, dst, sem, n = resident[key]
        rows = src.shape[0] // n
        for i in range(n):
            piece = pl.ds(i * rows, rows)
            pltpu.make_async_copy(src.at[piece], dst.at[piece], sem).start(priority=i % 2)

    def fetched(*key):
        src, dst, sem, _ = resident[key]
        pltpu.make_async_copy(src, dst, sem).wait()

    def ocopy_early():
        return pltpu.make_async_copy(o_early, out_hbm.at[pl.ds(0, nb - 1)], osem.at[0])

    def ocopy_last():
        return pltpu.make_async_copy(o_last, out_hbm.at[nb - 1], osem.at[1])

    def issue(t):
        kcopy(1, t).start(priority=0)
        if isinstance(t, int):
            if t + 1 < nt:
                kcopy(0, t + 1).start(priority=0)
        else:
            @pl.when(t + 1 < nt)
            def _():
                kcopy(0, t + 1).start(priority=0)
        vcopy(0, t).start(priority=1)
        vcopy(1, t).start(priority=1)

    def head_cols(t):
        return pl.ds(pl.multiple_of((t % nh) * _DH, _DH), _DH)

    def scores(br, t):
        x = x_buf[br, t // nh]
        wq = wq_buf[br, :, head_cols(t)]
        q = jnp.dot(x, wq, preferred_element_type=jnp.float32)
        q = (q * qscale).astype(jnp.bfloat16)
        k = k_buf[t % _NS, br]
        return lax.dot_general(q, k, (((1,), (1,)), ((), ())),
                               preferred_element_type=jnp.float32)

    def attend(br, t, s):
        m = jnp.max(s, axis=-1, keepdims=True)
        p = jnp.exp2(s - m)
        l = jnp.sum(p, axis=-1, keepdims=True)
        v = v_buf[t % _NS, br]
        o = jnp.dot(p.astype(jnp.bfloat16), v, preferred_element_type=jnp.float32)
        o = (o * (1.0 / l)).astype(jnp.bfloat16)
        wo = wo_buf[br, head_cols(t), :]
        acc[:, br * d_model:(br + 1) * d_model] += jnp.dot(
            o, wo, preferred_element_type=jnp.float32)

    fetch("x", 0)
    fetch("wq", 0)
    kcopy(0, 0).start(priority=0)
    fetch("x", 1)
    fetch("wq", 1)
    fetch("wo", 0)
    fetch("wo", 1)
    for t0 in range(_PD):
        issue(t0)
    acc[...] = jnp.zeros_like(acc)
    fetched("x", 0)
    fetched("wq", 0)
    kcopy(0, 0).wait()
    s_buf[...] = scores(0, 0)
    fetched("x", 1)
    fetched("wq", 1)
    fetched("wo", 0)
    fetched("wo", 1)

    def body(t, last):
        if not last:
            @pl.when(t + _PD < nt)
            def _():
                issue(t + _PD)

            @pl.when(t == nt - 2)
            def _():
                ocopy_early().start()

        kcopy(1, t).wait()
        if not last:
            kcopy(0, t + 1).wait()
        vcopy(0, t).wait()
        vcopy(1, t).wait()

        s_a = s_buf[...]
        s_b = scores(1, t)
        attend(0, t, s_a)
        if not last:
            s_buf[...] = scores(0, t + 1)
        attend(1, t, s_b)

        if last:
            o_last[...] = acc[...].astype(o_last.dtype)
            ocopy_last().start()
        else:
            @pl.when(t % nh == nh - 1)
            def _():
                o_early[t // nh] = acc[...].astype(o_early.dtype)
                acc[...] = jnp.zeros_like(acc)

    def loop_body(t, carry):
        body(t, False)
        return carry

    lax.fori_loop(0, nt - 1, loop_body, 0)
    body(nt - 1, True)
    ocopy_early().wait()
    ocopy_last().wait()


@jax.jit
def pallas_concat_heads__mha_block_cached__gqa_block_cached__near_ridge_kernel(
    A_x: jax.Array,
    A_k_cache: jax.Array,
    A_v_cache: jax.Array,
    A_wq: jax.Array,
    A_wo: jax.Array,
    B_x: jax.Array,
    B_k_cache: jax.Array,
    B_v_cache: jax.Array,
    B_wq: jax.Array,
    B_wo: jax.Array,
):
    nb, sq, d_model = A_x.shape
    sk = A_k_cache.shape[2]
    nh = A_wq.shape[1] // _DH
    assert B_x.shape == A_x.shape and B_wq.shape == A_wq.shape and B_wo.shape == A_wo.shape
    assert A_k_cache.shape == (nb, nh, sk, _DH) and A_v_cache.shape == A_k_cache.shape
    assert B_k_cache.shape[2:] == (sk, _DH) and B_v_cache.shape == B_k_cache.shape
    assert nh % B_k_cache.shape[1] == 0 and nb >= 2 and nh >= 2
    reps = (1, nh // B_k_cache.shape[1])
    dt = A_x.dtype

    kernel = functools.partial(_kernel, nb=nb, nh=nh, d_model=d_model, reps=reps)
    return pl.pallas_call(
        kernel,
        in_specs=[pl.BlockSpec(memory_space=pl.ANY)] * 10,
        out_specs=pl.BlockSpec(memory_space=pl.ANY),
        out_shape=jax.ShapeDtypeStruct((nb, sq, 2 * d_model), dt),
        scratch_shapes=[
            pltpu.VMEM((2, nb, sq, d_model), dt),
            pltpu.VMEM((2, d_model, nh * _DH), dt),
            pltpu.VMEM((2, nh * _DH, d_model), dt),
            pltpu.VMEM((_NS, 2, sk, _DH), dt),
            pltpu.VMEM((_NS, 2, sk, _DH), dt),
            pltpu.VMEM((sq, sk), jnp.float32),
            pltpu.VMEM((sq, 2 * d_model), jnp.float32),
            pltpu.VMEM((nb - 1, sq, 2 * d_model), dt),
            pltpu.VMEM((sq, 2 * d_model), dt),
            pltpu.SemaphoreType.DMA((6,)),
            pltpu.SemaphoreType.DMA((_NS, 2)),
            pltpu.SemaphoreType.DMA((_NS, 2)),
            pltpu.SemaphoreType.DMA((2,)),
        ],
        compiler_params=pltpu.CompilerParams(vmem_limit_bytes=64 * 1024 * 1024),
    )(A_x, A_k_cache, A_v_cache, A_wq, A_wo, B_x, B_k_cache, B_v_cache, B_wq, B_wo)
```
